```python
import os as _os
_os.environ.setdefault("JAX_PLATFORMS", "cpu")
import jax
import jax.numpy as jnp

def _softmax(x, axis=-1):
    return jax.nn.softmax(x, axis=axis)
def _gelu(x):
    return jax.nn.gelu(x, approximate=True)
def _silu(x):
    return jax.nn.silu(x)
def _sigmoid(x):
    return jax.nn.sigmoid(x)
def _layernorm(x, axis=-1, eps=1e-5):
    m = jnp.mean(x, axis=axis, keepdims=True)
    v = jnp.var(x, axis=axis, keepdims=True)
    return (x - m) / jnp.sqrt(v + eps)
def _scatter_add(tgt, idx, src, axis=0):
    return tgt.at[idx].add(src)
def _segment_sum(src, seg, n):
    return jax.ops.segment_sum(src, seg, n)
class _Rng:
    def __init__(self, key):
        self._k = key
    def _next(self):
        self._k, sub = jax.random.split(self._k)
        return sub
    def normal(self, shape):
        return jax.random.normal(self._next(), shape, dtype=jnp.bfloat16)
    def randint(self, lo, hi, shape):
        return jax.random.randint(self._next(), shape, lo, hi, dtype=jnp.int32)
    def uniform(self, shape, lo=0.0, hi=1.0):
        return jax.random.uniform(self._next(), shape, jnp.bfloat16, lo, hi)
    def permutation(self, n):
        return jax.random.permutation(self._next(), n)


kernel_name = 'concat_heads__mha_block_cached__mha_block_cached__near_ridge'

def setup_inputs():
    _rng = _Rng(jax.random.key(int.from_bytes(__import__("os").urandom(4), "little")))
    _w = (lambda a: (lambda t: t.astype(jnp.bfloat16) if jnp.issubdtype(t.dtype, jnp.floating) else t)(jnp.asarray(a)))
    def _A_setup():
        B, Sq, D = 32, 32, 640
        H, Sk, Dh = 32, 32, 128
        return {
            "x": _w((lambda *s: _rng.normal(s) * 0.8)(B, Sq, D)),
            "k_cache": _w((lambda *s: _rng.normal(s) * 0.8)(B, H, Sk, Dh)),
            "v_cache": _w((lambda *s: _rng.normal(s) * 0.05)(B, H, Sk, Dh)),
            "wq": _w((lambda *s: _rng.normal(s) * 0.8)(D, H * Dh) * (D ** -0.5)),
            "wo": _w((lambda *s: _rng.normal(s) * 0.05)(H * Dh, D) * ((H * Dh) ** -0.5)),
        }
    _A_in = _A_setup()

    def _B_setup():
        B, Sq, D = 32, 32, 640
        H, Sk, Dh = 32, 32, 128
        return {
            "x": _w((lambda *s: _rng.normal(s) * 0.8)(B, Sq, D)),
            "k_cache": _w((lambda *s: _rng.normal(s) * 0.8)(B, H, Sk, Dh)),
            "v_cache": _w((lambda *s: _rng.normal(s) * 0.05)(B, H, Sk, Dh)),
            "wq": _w((lambda *s: _rng.normal(s) * 0.8)(D, H * Dh) * (D ** -0.5)),
            "wo": _w((lambda *s: _rng.normal(s) * 0.05)(H * Dh, D) * ((H * Dh) ** -0.5)),
        }
    _B_in = _B_setup()

    return {
        "A_x": _A_in["x"],
        "A_k_cache": _A_in["k_cache"],
        "A_v_cache": _A_in["v_cache"],
        "A_wq": _A_in["wq"],
        "A_wo": _A_in["wo"],
        "B_x": _B_in["x"],
        "B_k_cache": _B_in["k_cache"],
        "B_v_cache": _B_in["v_cache"],
        "B_wq": _B_in["wq"],
        "B_wo": _B_in["wo"],
    }

def reference(A_x, A_k_cache, A_v_cache, A_wq, A_wo, B_x, B_k_cache, B_v_cache, B_wq, B_wo):
    def _A_ref(x, k_cache, v_cache, wq, wo):
        B, Sq, D = x.shape
        H, Dh = 32, 128
        q = (lambda x, *d: x.transpose(*d))((x @ wq).reshape(B, Sq, H, Dh), 0, 2, 1, 3)
        scores = jnp.einsum("bhqd,bhkd->bhqk", q, k_cache) * (Dh ** -0.5)
        p = _softmax(scores, axis=-1)
        o = jnp.einsum("bhqk,bhkd->bhqd", p, v_cache)
        return (lambda x, *d: x.transpose(*d))(o, 0, 2, 1, 3).reshape(B, Sq, H * Dh) @ wo

    def _B_ref(x, k_cache, v_cache, wq, wo):
        B, Sq, D = x.shape
        H, Dh = 32, 128
        q = (lambda x, *d: x.transpose(*d))((x @ wq).reshape(B, Sq, H, Dh), 0, 2, 1, 3)
        scores = jnp.einsum("bhqd,bhkd->bhqk", q, k_cache) * (Dh ** -0.5)
        p = _softmax(scores, axis=-1)
        o = jnp.einsum("bhqk,bhkd->bhqd", p, v_cache)
        return (lambda x, *d: x.transpose(*d))(o, 0, 2, 1, 3).reshape(B, Sq, H * Dh) @ wo

    a = _A_ref(A_x, A_k_cache, A_v_cache, A_wq, A_wo)
    b = _B_ref(B_x, B_k_cache, B_v_cache, B_wq, B_wo)
    return jnp.concatenate([a, b], axis=-1)
```

```python
import math
import jax
import jax.numpy as jnp
from jax import lax
import jax.experimental.pallas as pl
import jax.experimental.pallas.tpu as pltpu

UNROLL = 2
XCH = 4
OCH = 4
B, SQ, D = 32, 32, 640
H, SK, DH = 32, 32, 128
M = B * SQ
HC = 4
NSTEP = H // HC
NT = 2 * NSTEP
GB = 4
NG = B // GB
CW = HC * DH
EXP2_SCALE = (DH ** -0.5) * math.log2(math.e)

S_WQ, S_K, S_V, S_WO, S_XB, S_OA = 0, 2, 4, 6, 8, 9
S_XA = 10
S_OB = S_XA + XCH
NSEM = S_OB + OCH

import contextlib
def scope(name):
    return contextlib.nullcontext()


def _kernel(ax, ak, av, awq, awo, bx, bk, bv, bwq, bwo, out_hbm,
            x_buf, wq_buf, wo_buf, k_buf, v_buf, q_scr, o_scr, acc, out_buf, sems):
    A = (ax, ak, av, awq, awo)
    Bq = (bx, bk, bv, bwq, bwo)

    def chunk_copy(refs, jj, sl, kind):
        _, k, v, wq, wo = refs
        if isinstance(jj, int):
            c0 = jj * CW
        else:
            c0 = pl.multiple_of(jj * CW, CW)
        h0 = jj * HC
        if kind == "wq":
            return pltpu.make_async_copy(wq.at[:, pl.ds(c0, CW)], wq_buf.at[sl], sems.at[S_WQ + sl])
        if kind == "k":
            return pltpu.make_async_copy(k.at[:, pl.ds(h0, HC)], k_buf.at[sl], sems.at[S_K + sl])
        if kind == "v":
            return pltpu.make_async_copy(v.at[:, pl.ds(h0, HC)], v_buf.at[sl], sems.at[S_V + sl])
        return pltpu.make_async_copy(wo.at[pl.ds(c0, CW), :], wo_buf.at[sl], sems.at[S_WO + sl])

    def dma(kind, t, sl, op):
        if isinstance(t, int):
            refs, jj = (A, t) if t < NSTEP else (Bq, t - NSTEP)
            getattr(chunk_copy(refs, jj, sl, kind), op)()
        else:
            @pl.when(t < NSTEP)
            def _():
                getattr(chunk_copy(A, t, sl, kind), op)()

            @pl.when(t >= NSTEP)
            def _():
                getattr(chunk_copy(Bq, t - NSTEP, sl, kind), op)()

    XR = M // XCH
    def xa_copy(c):
        return pltpu.make_async_copy(ax.at[pl.ds(c * XR, XR)], x_buf.at[0, pl.ds(c * XR, XR)], sems.at[S_XA + c])

    def xb_copy():
        return pltpu.make_async_copy(bx, x_buf.at[1], sems.at[S_XB])

    def outa_copy():
        return pltpu.make_async_copy(out_buf.at[0], out_hbm.at[:, pl.ds(0, D)], sems.at[S_OA])

    OR = M // OCH
    def outb_copy(c):
        return pltpu.make_async_copy(out_buf.at[1, pl.ds(c * OR, OR)],
                                     out_hbm.at[pl.ds(c * OR, OR), pl.ds(D, D)], sems.at[S_OB + c])

    rb = lax.broadcasted_iota(jnp.int32, (128, 128), 0) // SQ
    cb = lax.broadcasted_iota(jnp.int32, (128, 128), 1) // SK
    mask = rb == cb
    units = [(h, g) for h in range(HC) for g in range(NG)]

    def qproj(t, sl):
        x = x_buf[t // NSTEP]
        q = jnp.dot(x, wq_buf[sl], preferred_element_type=jnp.float32)
        q_scr[sl] = q.astype(jnp.bfloat16)

    def scores_softmax(sl):
        ps = []
        for (h, g) in units:
            qg = q_scr[sl, g * 128:(g + 1) * 128, h * DH:(h + 1) * DH]
            kg = k_buf[sl, g * GB:(g + 1) * GB, h].reshape(128, DH)
            sc = lax.dot_general(qg, kg, (((1,), (1,)), ((), ())),
                                 preferred_element_type=jnp.float32)
            sc = jnp.where(mask, sc, -jnp.inf)
            m = jnp.max(sc, axis=-1, keepdims=True)
            p = jnp.exp2((sc - m) * EXP2_SCALE)
            l = jnp.sum(p, axis=-1, keepdims=True)
            r = pl.reciprocal(l, approx=True)
            r = r * (2.0 - l * r)
            ps.append((p * r).astype(jnp.bfloat16))
        return ps

    def pv(sl, ps):
        for (h, g), p in zip(units, ps):
            vg = v_buf[sl, g * GB:(g + 1) * GB, h].reshape(128, DH)
            o = jnp.dot(p, vg, preferred_element_type=jnp.float32)
            o_scr[sl, g * 128:(g + 1) * 128, h * DH:(h + 1) * DH] = o.astype(jnp.bfloat16)

    def oproj(t, sl):
        b = t // NSTEP
        acc[b] += jnp.dot(o_scr[sl], wo_buf[sl], preferred_element_type=jnp.float32)

    def step(t, sl):
        ps_ = 1 - sl

        @pl.when(t + 1 < NT)
        def _():
            dma("wq", t + 1, ps_, "start")
        dma("k", t, sl, "start")
        dma("wo", t - 1, ps_, "start")
        dma("v", t, sl, "start")
        dma("k", t - 1, ps_, "wait")
        dma("wo", t - 2, sl, "wait")
        dma("wq", t, sl, "wait")
        dma("v", t - 1, ps_, "wait")
        ps = scores_softmax(ps_)
        oproj(t - 2, sl)
        qproj(t, sl)
        pv(ps_, ps)

    dma("wq", 0, 0, "start")
    for c in range(XCH):
        xa_copy(c).start()
    dma("k", 0, 0, "start")
    dma("wq", 1, 1, "start")
    dma("v", 0, 0, "start")
    with scope("step0"):
        dma("wq", 0, 0, "wait")
        for c in range(XCH):
            xa_copy(c).wait()
            q = jnp.dot(x_buf[0, c * XR:(c + 1) * XR], wq_buf[0], preferred_element_type=jnp.float32)
            q_scr[0, c * XR:(c + 1) * XR] = q.astype(jnp.bfloat16)
    with scope("step1"):
        dma("wq", 2, 0, "start")
        dma("k", 1, 1, "start")
        dma("wo", 0, 0, "start")
        dma("v", 1, 1, "start")
        dma("k", 0, 0, "wait")
        dma("wq", 1, 1, "wait")
        ps = scores_softmax(0)
        acc[...] = jnp.zeros(acc.shape, acc.dtype)
        qproj(1, 1)
        dma("v", 0, 0, "wait")
        pv(0, ps)

    def special(t):
        @pl.when(t == 3)
        def _():
            xb_copy().start()

        @pl.when(t == NSTEP)
        def _():
            xb_copy().wait()

        @pl.when(t == NSTEP + 2)
        def _():
            out_buf[0] = acc[0].astype(out_buf.dtype)
            outa_copy().start()

    def body(i, carry):
        for u in range(UNROLL):
            t = 2 + i * UNROLL + u
            special(t)
            with scope("loopstep"):
                step(t, u if UNROLL == 2 else t % 2)
        return carry

    lax.fori_loop(0, (NT - 2) // UNROLL, body, 0)

    with scope("step16"):
        dma("wo", NT - 1, 1, "start")
        dma("k", NT - 1, 1, "wait")
        dma("wo", NT - 2, 0, "wait")
        dma("v", NT - 1, 1, "wait")
        ps = scores_softmax(1)
        oproj(NT - 2, 0)
        pv(1, ps)
        dma("wo", NT - 1, 1, "wait")
        for c in range(OCH):
            rows = slice(c * OR, (c + 1) * OR)
            res = acc[1, rows] + jnp.dot(o_scr[1, rows], wo_buf[1], preferred_element_type=jnp.float32)
            out_buf[1, rows] = res.astype(out_buf.dtype)
            outb_copy(c).start()
    with scope("final"):
        outa_copy().wait()
        for c in range(OCH):
            outb_copy(c).wait()


@jax.jit
def pallas_concat_heads__mha_block_cached__mha_block_cached__near_ridge_kernel(
    A_x, A_k_cache, A_v_cache, A_wq, A_wo, B_x, B_k_cache, B_v_cache, B_wq, B_wo,
):
    ax = A_x.reshape(M, D)
    bx = B_x.reshape(M, D)
    bf = jnp.bfloat16
    out = pl.pallas_call(
        _kernel,
        in_specs=[pl.BlockSpec(memory_space=pl.ANY)] * 10,
        out_specs=pl.BlockSpec(memory_space=pl.ANY),
        out_shape=jax.ShapeDtypeStruct((M, 2 * D), bf),
        scratch_shapes=[
            pltpu.VMEM((2, M, D), bf),
            pltpu.VMEM((2, D, CW), bf),
            pltpu.VMEM((2, CW, D), bf),
            pltpu.VMEM((2, B, HC, SK, DH), bf),
            pltpu.VMEM((2, B, HC, SK, DH), bf),
            pltpu.VMEM((2, M, CW), bf),
            pltpu.VMEM((2, M, CW), bf),
            pltpu.VMEM((2, M, D), jnp.float32),
            pltpu.VMEM((2, M, D), bf),
            pltpu.SemaphoreType.DMA((NSEM,)),
        ],
        compiler_params=pltpu.CompilerParams(
            vmem_limit_bytes=96 * 1024 * 1024, disable_bounds_checks=True,
        ),
    )(ax, A_k_cache, A_v_cache, A_wq, A_wo, bx, B_k_cache, B_v_cache, B_wq, B_wo)
    return out.reshape(B, SQ, 2 * D)
```

```python
import math

import jax
import jax.numpy as jnp
from jax import lax
import jax.experimental.pallas as pl
import jax.experimental.pallas.tpu as pltpu

B, SQ, D = 32, 32, 640
H, SK, DH = 32, 32, 128
M = B * SQ
HC = 4
NSTEP = H // HC
NT = 2 * NSTEP
GB = 4
NG = B // GB
CW = HC * DH
XCH = 4
OCH = 8
XR = M // XCH
OR = M // OCH
EXP2_SCALE = (DH ** -0.5) * math.log2(math.e)

S_WQ, S_K, S_V, S_WO, S_XB, S_OA = 0, 2, 4, 6, 8, 9
S_XA = 10
S_OB = S_XA + XCH
NSEM = S_OB + OCH


def _kernel(ax, ak, av, awq, awo, bx, bk, bv, bwq, bwo, out_hbm,
            x_buf, wq_buf, wo_buf, k_buf, v_buf, q_scr, o_scr, acc, out_buf, sems):
    blk_a = (ak, av, awq, awo)
    blk_b = (bk, bv, bwq, bwo)

    def chunk_copy(refs, jj, sl, kind):
        k, v, wq, wo = refs
        c0 = jj * CW if isinstance(jj, int) else pl.multiple_of(jj * CW, CW)
        h0 = jj * HC
        if kind == "wq":
            return pltpu.make_async_copy(wq.at[:, pl.ds(c0, CW)], wq_buf.at[sl], sems.at[S_WQ + sl])
        if kind == "k":
            return pltpu.make_async_copy(k.at[:, pl.ds(h0, HC)], k_buf.at[sl], sems.at[S_K + sl])
        if kind == "v":
            return pltpu.make_async_copy(v.at[:, pl.ds(h0, HC)], v_buf.at[sl], sems.at[S_V + sl])
        return pltpu.make_async_copy(wo.at[pl.ds(c0, CW), :], wo_buf.at[sl], sems.at[S_WO + sl])

    def dma(kind, t, sl, op):
        if isinstance(t, int):
            refs, jj = (blk_a, t) if t < NSTEP else (blk_b, t - NSTEP)
            getattr(chunk_copy(refs, jj, sl, kind), op)()
        else:
            @pl.when(t < NSTEP)
            def _():
                getattr(chunk_copy(blk_a, t, sl, kind), op)()

            @pl.when(t >= NSTEP)
            def _():
                getattr(chunk_copy(blk_b, t - NSTEP, sl, kind), op)()

    def xa_copy(c):
        return pltpu.make_async_copy(ax.at[pl.ds(c * XR, XR)], x_buf.at[0, pl.ds(c * XR, XR)],
                                     sems.at[S_XA + c])

    def xb_copy():
        return pltpu.make_async_copy(bx, x_buf.at[1], sems.at[S_XB])

    def outa_copy():
        return pltpu.make_async_copy(out_buf.at[0], out_hbm.at[:, pl.ds(0, D)], sems.at[S_OA])

    def outb_copy(c):
        return pltpu.make_async_copy(out_buf.at[1, pl.ds(c * OR, OR)],
                                     out_hbm.at[pl.ds(c * OR, OR), pl.ds(D, D)], sems.at[S_OB + c])

    row_b = lax.broadcasted_iota(jnp.int32, (128, 128), 0) // SQ
    col_b = lax.broadcasted_iota(jnp.int32, (128, 128), 1) // SK
    mask = row_b == col_b
    units = [(h, g) for h in range(HC) for g in range(NG)]

    def qproj(t, sl):
        q = jnp.dot(x_buf[t // NSTEP], wq_buf[sl], preferred_element_type=jnp.float32)
        q_scr[sl] = q.astype(jnp.bfloat16)

    def scores_softmax(sl):
        ps = []
        for (h, g) in units:
            qg = q_scr[sl, g * 128:(g + 1) * 128, h * DH:(h + 1) * DH]
            kg = k_buf[sl, g * GB:(g + 1) * GB, h].reshape(128, DH)
            sc = lax.dot_general(qg, kg, (((1,), (1,)), ((), ())),
                                 preferred_element_type=jnp.float32)
            sc = jnp.where(mask, sc, -jnp.inf)
            m = jnp.max(sc, axis=-1, keepdims=True)
            p = jnp.exp2((sc - m) * EXP2_SCALE)
            l = jnp.sum(p, axis=-1, keepdims=True)
            r = pl.reciprocal(l, approx=True)
            r = r * (2.0 - l * r)
            ps.append((p * r).astype(jnp.bfloat16))
        return ps

    def pv(sl, ps):
        for (h, g), p in zip(units, ps):
            vg = v_buf[sl, g * GB:(g + 1) * GB, h].reshape(128, DH)
            o = jnp.dot(p, vg, preferred_element_type=jnp.float32)
            o_scr[sl, g * 128:(g + 1) * 128, h * DH:(h + 1) * DH] = o.astype(jnp.bfloat16)

    def oproj(t, sl):
        acc[t // NSTEP] += jnp.dot(o_scr[sl], wo_buf[sl], preferred_element_type=jnp.float32)

    def step(t, sl):
        ps_ = 1 - sl

        @pl.when(t + 1 < NT)
        def _():
            dma("wq", t + 1, ps_, "start")
        dma("k", t, sl, "start")
        dma("wo", t - 1, ps_, "start")
        dma("v", t, sl, "start")
        dma("k", t - 1, ps_, "wait")
        dma("wo", t - 2, sl, "wait")
        dma("wq", t, sl, "wait")
        dma("v", t - 1, ps_, "wait")
        ps = scores_softmax(ps_)
        oproj(t - 2, sl)
        qproj(t, sl)
        pv(ps_, ps)

    dma("wq", 0, 0, "start")
    for c in range(XCH):
        xa_copy(c).start()
    dma("k", 0, 0, "start")
    dma("wq", 1, 1, "start")
    dma("v", 0, 0, "start")
    acc[...] = jnp.zeros(acc.shape, acc.dtype)
    dma("wq", 0, 0, "wait")
    for c in range(XCH):
        xa_copy(c).wait()
        q = jnp.dot(x_buf[0, c * XR:(c + 1) * XR], wq_buf[0], preferred_element_type=jnp.float32)
        q_scr[0, c * XR:(c + 1) * XR] = q.astype(jnp.bfloat16)

    dma("wq", 2, 0, "start")
    dma("k", 1, 1, "start")
    dma("wo", 0, 0, "start")
    dma("v", 1, 1, "start")
    dma("k", 0, 0, "wait")
    dma("wq", 1, 1, "wait")
    ps = scores_softmax(0)
    qproj(1, 1)
    dma("v", 0, 0, "wait")
    pv(0, ps)

    def special(t):
        @pl.when(t == 3)
        def _():
            xb_copy().start()

        @pl.when(t == NSTEP)
        def _():
            xb_copy().wait()

        @pl.when(t == NSTEP + 2)
        def _():
            out_buf[0] = acc[0].astype(out_buf.dtype)
            outa_copy().start()

    def body(i, carry):
        for u in range(2):
            t = 2 + i * 2 + u
            special(t)
            step(t, u)
        return carry

    lax.fori_loop(0, (NT - 2) // 2, body, 0)

    dma("wo", NT - 1, 1, "start")
    dma("k", NT - 1, 1, "wait")
    dma("wo", NT - 2, 0, "wait")
    dma("v", NT - 1, 1, "wait")
    ps = scores_softmax(1)
    oproj(NT - 2, 0)
    pv(1, ps)
    dma("wo", NT - 1, 1, "wait")
    for c in range(OCH):
        rows = slice(c * OR, (c + 1) * OR)
        res = acc[1, rows] + jnp.dot(o_scr[1, rows], wo_buf[1], preferred_element_type=jnp.float32)
        out_buf[1, rows] = res.astype(out_buf.dtype)
        outb_copy(c).start()
    outa_copy().wait()
    for c in range(OCH):
        outb_copy(c).wait()


@jax.jit
def pallas_concat_heads__mha_block_cached__mha_block_cached__near_ridge_kernel(
    A_x: jax.Array,
    A_k_cache: jax.Array,
    A_v_cache: jax.Array,
    A_wq: jax.Array,
    A_wo: jax.Array,
    B_x: jax.Array,
    B_k_cache: jax.Array,
    B_v_cache: jax.Array,
    B_wq: jax.Array,
    B_wo: jax.Array,
):
    bf = jnp.bfloat16
    out = pl.pallas_call(
        _kernel,
        in_specs=[pl.BlockSpec(memory_space=pl.ANY)] * 10,
        out_specs=pl.BlockSpec(memory_space=pl.ANY),
        out_shape=jax.ShapeDtypeStruct((M, 2 * D), bf),
        scratch_shapes=[
            pltpu.VMEM((2, M, D), bf),
            pltpu.VMEM((2, D, CW), bf),
            pltpu.VMEM((2, CW, D), bf),
            pltpu.VMEM((2, B, HC, SK, DH), bf),
            pltpu.VMEM((2, B, HC, SK, DH), bf),
            pltpu.VMEM((2, M, CW), bf),
            pltpu.VMEM((2, M, CW), bf),
            pltpu.VMEM((2, M, D), jnp.float32),
            pltpu.VMEM((2, M, D), bf),
            pltpu.SemaphoreType.DMA((NSEM,)),
        ],
        compiler_params=pltpu.CompilerParams(
            vmem_limit_bytes=96 * 1024 * 1024,
            disable_bounds_checks=True,
        ),
    )(A_x.reshape(M, D), A_k_cache, A_v_cache, A_wq, A_wo,
      B_x.reshape(M, D), B_k_cache, B_v_cache, B_wq, B_wo)
    return out.reshape(B, SQ, 2 * D)
```

```python
import math

import jax
import jax.numpy as jnp
from jax import lax
import jax.experimental.pallas as pl
import jax.experimental.pallas.tpu as pltpu

B, SQ, D = 32, 32, 640
H, SK, DH = 32, 32, 128
M = B * SQ
HC = 4
NSTEP = H // HC
NT = 2 * NSTEP
GB = 4
NG = B // GB
CW = HC * DH
XCH = 4
OCH = 8
XR = M // XCH
OR = M // OCH
EXP2_SCALE = (DH ** -0.5) * math.log2(math.e)

S_WQ, S_K, S_V, S_WO, S_XB, S_OA = 0, 2, 4, 6, 8, 9
S_XA = 10
S_OB = S_XA + XCH
NSEM = S_OB + OCH


def _kernel(ax, ak, av, awq, awo, bx, bk, bv, bwq, bwo, out_hbm,
            x_buf, wq_buf, wo_buf, k_buf, v_buf, q_scr, o_scr, acc, out_buf, sems):
    blk_a = (ak, av, awq, awo)
    blk_b = (bk, bv, bwq, bwo)

    def chunk_copy(refs, jj, sl, kind):
        k, v, wq, wo = refs
        c0 = jj * CW if isinstance(jj, int) else pl.multiple_of(jj * CW, CW)
        h0 = jj * HC
        if kind == "wq":
            return pltpu.make_async_copy(wq.at[:, pl.ds(c0, CW)], wq_buf.at[sl], sems.at[S_WQ + sl])
        if kind == "k":
            return pltpu.make_async_copy(k.at[:, pl.ds(h0, HC)], k_buf.at[sl], sems.at[S_K + sl])
        if kind == "v":
            return pltpu.make_async_copy(v.at[:, pl.ds(h0, HC)], v_buf.at[sl], sems.at[S_V + sl])
        return pltpu.make_async_copy(wo.at[pl.ds(c0, CW), :], wo_buf.at[sl], sems.at[S_WO + sl])

    def dma(kind, t, sl, op):
        if isinstance(t, int):
            refs, jj = (blk_a, t) if t < NSTEP else (blk_b, t - NSTEP)
            getattr(chunk_copy(refs, jj, sl, kind), op)()
        else:
            @pl.when(t < NSTEP)
            def _():
                getattr(chunk_copy(blk_a, t, sl, kind), op)()

            @pl.when(t >= NSTEP)
            def _():
                getattr(chunk_copy(blk_b, t - NSTEP, sl, kind), op)()

    def xa_copy(c):
        return pltpu.make_async_copy(ax.at[pl.ds(c * XR, XR)], x_buf.at[0, pl.ds(c * XR, XR)],
                                     sems.at[S_XA + c])

    def xb_copy():
        return pltpu.make_async_copy(bx, x_buf.at[1], sems.at[S_XB])

    def outa_copy():
        return pltpu.make_async_copy(out_buf.at[0], out_hbm.at[:, pl.ds(0, D)], sems.at[S_OA])

    def outb_copy(c):
        return pltpu.make_async_copy(out_buf.at[1, pl.ds(c * OR, OR)],
                                     out_hbm.at[pl.ds(c * OR, OR), pl.ds(D, D)], sems.at[S_OB + c])

    row_b = lax.broadcasted_iota(jnp.int32, (128, 128), 0) // SQ
    col_b = lax.broadcasted_iota(jnp.int32, (128, 128), 1) // SK
    mask = row_b == col_b
    units = [(h, g) for h in range(HC) for g in range(NG)]

    def qproj(t, sl):
        q = jnp.dot(x_buf[t // NSTEP], wq_buf[sl], preferred_element_type=jnp.float32)
        q_scr[sl] = q.astype(jnp.bfloat16)

    def scores_softmax(sl):
        ps = []
        for (h, g) in units:
            qg = q_scr[sl, g * 128:(g + 1) * 128, h * DH:(h + 1) * DH]
            kg = k_buf[sl, g * GB:(g + 1) * GB, h].reshape(128, DH)
            sc = lax.dot_general(qg, kg, (((1,), (1,)), ((), ())),
                                 preferred_element_type=jnp.float32)
            sc = jnp.where(mask, sc, -jnp.inf)
            m = jnp.max(sc, axis=-1, keepdims=True)
            p = jnp.exp2((sc - m) * EXP2_SCALE)
            l = jnp.sum(p, axis=-1, keepdims=True)
            r = pl.reciprocal(l, approx=True)
            r = r * (2.0 - l * r)
            ps.append((p * r).astype(jnp.bfloat16))
        return ps

    def pv(sl, ps):
        for (h, g), p in zip(units, ps):
            vg = v_buf[sl, g * GB:(g + 1) * GB, h].reshape(128, DH)
            o = jnp.dot(p, vg, preferred_element_type=jnp.float32)
            o_scr[sl, g * 128:(g + 1) * 128, h * DH:(h + 1) * DH] = o.astype(jnp.bfloat16)

    def oproj(t, sl):
        b = t // NSTEP
        res = acc[b] + jnp.dot(o_scr[sl], wo_buf[sl], preferred_element_type=jnp.float32)
        acc[b] = res
        if not isinstance(t, int):
            out_buf[b] = res.astype(out_buf.dtype)

    def step(t, sl):
        ps_ = 1 - sl

        @pl.when(t + 1 < NT)
        def _():
            dma("wq", t + 1, ps_, "start")
        dma("k", t, sl, "start")
        dma("wo", t - 1, ps_, "start")
        dma("v", t, sl, "start")
        dma("k", t - 1, ps_, "wait")
        dma("wo", t - 2, sl, "wait")
        dma("wq", t, sl, "wait")
        dma("v", t - 1, ps_, "wait")
        ps = scores_softmax(ps_)
        oproj(t - 2, sl)
        qproj(t, sl)
        pv(ps_, ps)

    dma("wq", 0, 0, "start")
    for c in range(XCH):
        xa_copy(c).start()
    dma("k", 0, 0, "start")
    dma("wq", 1, 1, "start")
    dma("v", 0, 0, "start")
    acc[...] = jnp.zeros(acc.shape, acc.dtype)
    dma("wq", 0, 0, "wait")
    for c in range(XCH):
        xa_copy(c).wait()
        q = jnp.dot(x_buf[0, c * XR:(c + 1) * XR], wq_buf[0], preferred_element_type=jnp.float32)
        q_scr[0, c * XR:(c + 1) * XR] = q.astype(jnp.bfloat16)

    dma("wq", 2, 0, "start")
    dma("k", 1, 1, "start")
    dma("wo", 0, 0, "start")
    dma("v", 1, 1, "start")
    dma("k", 0, 0, "wait")
    dma("wq", 1, 1, "wait")
    ps = scores_softmax(0)
    qproj(1, 1)
    dma("v", 0, 0, "wait")
    pv(0, ps)

    def special(t):
        @pl.when(t == 4)
        def _():
            xb_copy().start()

        @pl.when(t == NSTEP)
        def _():
            xb_copy().wait()

        @pl.when(t == NSTEP + 2)
        def _():
            outa_copy().start()

    def body(i, carry):
        for u in range(2):
            t = 2 + i * 2 + u
            if u == 0:
                special(t)
            step(t, u)
        return carry

    lax.fori_loop(0, (NT - 2) // 2, body, 0)

    dma("wo", NT - 1, 1, "start")
    dma("k", NT - 1, 1, "wait")
    dma("wo", NT - 2, 0, "wait")
    dma("v", NT - 1, 1, "wait")
    ps = scores_softmax(1)
    oproj(NT - 2, 0)
    pv(1, ps)
    dma("wo", NT - 1, 1, "wait")
    for c in range(OCH):
        rows = slice(c * OR, (c + 1) * OR)
        res = acc[1, rows] + jnp.dot(o_scr[1, rows], wo_buf[1], preferred_element_type=jnp.float32)
        out_buf[1, rows] = res.astype(out_buf.dtype)
        outb_copy(c).start()
    outa_copy().wait()
    for c in range(OCH):
        outb_copy(c).wait()


@jax.jit
def pallas_concat_heads__mha_block_cached__mha_block_cached__near_ridge_kernel(
    A_x: jax.Array,
    A_k_cache: jax.Array,
    A_v_cache: jax.Array,
    A_wq: jax.Array,
    A_wo: jax.Array,
    B_x: jax.Array,
    B_k_cache: jax.Array,
    B_v_cache: jax.Array,
    B_wq: jax.Array,
    B_wo: jax.Array,
):
    bf = jnp.bfloat16
    out = pl.pallas_call(
        _kernel,
        in_specs=[pl.BlockSpec(memory_space=pl.ANY)] * 10,
        out_specs=pl.BlockSpec(memory_space=pl.ANY),
        out_shape=jax.ShapeDtypeStruct((M, 2 * D), bf),
        scratch_shapes=[
            pltpu.VMEM((2, M, D), bf),
            pltpu.VMEM((2, D, CW), bf),
            pltpu.VMEM((2, CW, D), bf),
            pltpu.VMEM((2, B, HC, SK, DH), bf),
            pltpu.VMEM((2, B, HC, SK, DH), bf),
            pltpu.VMEM((2, M, CW), bf),
            pltpu.VMEM((2, M, CW), bf),
            pltpu.VMEM((2, M, D), jnp.float32),
            pltpu.VMEM((2, M, D), bf),
            pltpu.SemaphoreType.DMA((NSEM,)),
        ],
        compiler_params=pltpu.CompilerParams(
            vmem_limit_bytes=96 * 1024 * 1024,
            disable_bounds_checks=True,
        ),
    )(A_x.reshape(M, D), A_k_cache, A_v_cache, A_wq, A_wo,
      B_x.reshape(M, D), B_k_cache, B_v_cache, B_wq, B_wo)
    return out.reshape(B, SQ, 2 * D)
```
